```python
import os as _os
_os.environ.setdefault("JAX_PLATFORMS", "cpu")
import jax
import jax.numpy as jnp

def _softmax(x, axis=-1):
    return jax.nn.softmax(x, axis=axis)
def _gelu(x):
    return jax.nn.gelu(x, approximate=True)
def _silu(x):
    return jax.nn.silu(x)
def _sigmoid(x):
    return jax.nn.sigmoid(x)
def _layernorm(x, axis=-1, eps=1e-5):
    m = jnp.mean(x, axis=axis, keepdims=True)
    v = jnp.var(x, axis=axis, keepdims=True)
    return (x - m) / jnp.sqrt(v + eps)
def _scatter_add(tgt, idx, src, axis=0):
    return tgt.at[idx].add(src)
def _segment_sum(src, seg, n):
    return jax.ops.segment_sum(src, seg, n)
class _Rng:
    def __init__(self, key):
        self._k = key
    def _next(self):
        self._k, sub = jax.random.split(self._k)
        return sub
    def normal(self, shape):
        return jax.random.normal(self._next(), shape, dtype=jnp.bfloat16)
    def randint(self, lo, hi, shape):
        return jax.random.randint(self._next(), shape, lo, hi, dtype=jnp.int32)
    def uniform(self, shape, lo=0.0, hi=1.0):
        return jax.random.uniform(self._next(), shape, jnp.bfloat16, lo, hi)
    def permutation(self, n):
        return jax.random.permutation(self._next(), n)


kernel_name = 'recurrent_scan__spectral_gfnet__swiglu_ffn__prompt'

def setup_inputs():
    _rng = _Rng(jax.random.key(int.from_bytes(__import__("os").urandom(4), "little")))
    _w = (lambda a: (lambda t: t.astype(jnp.bfloat16) if jnp.issubdtype(t.dtype, jnp.floating) else t)(jnp.asarray(a)))
    def _A_setup():
        B, S, D = 1, 2048, 640
        Df = D // 2 + 1
        return {
            "x": _w((lambda *s: _rng.normal(s) * 0.05)(B, S, D)),
            "w_r": _w((lambda *s: _rng.normal(s) * 0.05)(S, Df) * 0.02),
            "w_i": _w((lambda *s: _rng.normal(s) * 0.05)(S, Df) * 0.02),
        }
    _A_in = _A_setup()

    def _B_setup():
        B, S, D, F = 1, 2048, 640, 1536
        return {
            "x": _w((lambda *s: _rng.normal(s) * 0.05)(B, S, D)),
            "w_gate": _w((lambda *s: _rng.normal(s) * 0.05)(D, F)),
            "w_up": _w((lambda *s: _rng.normal(s) * 0.05)(D, F)),
            "w_down": _w((lambda *s: _rng.normal(s) * 0.05)(F, D)),
        }
    _B_in = _B_setup()

    return {
        "A_x": _A_in["x"],
        "A_w_r": _A_in["w_r"],
        "A_w_i": _A_in["w_i"],
        "B_x": _B_in["x"],
        "B_w_gate": _B_in["w_gate"],
        "B_w_up": _B_in["w_up"],
        "B_w_down": _B_in["w_down"],
    }

def reference(A_x, A_w_r, A_w_i, B_x, B_w_gate, B_w_up, B_w_down):
    def _A_ref(x, w_r, w_i):
        B, S, D = x.shape
        X = (lambda x, axes=(-2,-1): jnp.fft.rfft2(x.astype(jnp.float32), axes=axes))(x, axes=(-2, -1))
        W = w_r + 1j * w_i
        X = X * W
        y = (lambda x, s, axes=(-2,-1): jnp.fft.irfft2(x, s=s, axes=axes).astype(jnp.bfloat16))(X, (S, D), axes=(-2, -1))
        return y

    def _B_ref(x, w_gate, w_up, w_down):
        g = _silu(x @ w_gate)
        u = x @ w_up
        return (g * u) @ w_down

    x = A_x
    xn = _layernorm(x, axis=-1)
    s = _A_ref(xn, A_w_r, A_w_i)
    g = _silu(_B_ref(xn, B_w_gate, B_w_up, B_w_down))
    return x + s * g
```

```python
import numpy as np
import ml_dtypes
import jax
import jax.numpy as jnp
from jax.experimental import pallas as pl
from jax.experimental.pallas import tpu as pltpu

S, D = 2048, 640
R = 16
P = S // R
KR = 336
U32 = jnp.uint32
XS0 = 2 * R * KR
WS0 = XS0 + 5120
M_ROWS = WS0 + 1920
BF = jnp.bfloat16
F32 = jnp.float32


def _consts():
    bf = ml_dtypes.bfloat16
    i = np.arange(32)
    d0 = np.arange(128)[:, None]
    def cls(rs):
        k = np.concatenate([r + 10 * i for r in rs])
        sg = np.where((k % 5) <= 2, 1.0, -1.0)[None, :]
        a = 2 * np.pi * ((d0 * k[None, :]) % D) / D
        return np.cos(a), np.sin(a), sg
    fw = []
    for rs in ((1, 4, 6, 9), (2, 3, 7, 8)):
        c, s, sg = cls(rs)
        fw += [c.T, (c - sg * s).T, (c + sg * s).T]
    k = np.concatenate([10 * i, 5 + 10 * i, [320]])
    a = 2 * np.pi * ((d0 * k[None, :]) % D) / D
    wt = np.where((k == 0) | (k == 320), 0.5, 1.0)[None, :]
    c, s = np.cos(a), np.sin(a) * ((k != 0) & (k != 320))[None, :]
    f0 = np.zeros((160, 128)); f0[:65] = c.T; f0[80:145] = -s.T
    i0 = np.concatenate([(c * wt).T[:64], (c * wt).T[64:], -s.T[1:64]])
    s0 = np.arange(R)[:, None, None]; s1 = np.arange(P)[None, :, None]; q = np.arange(P)[None, None, :]
    a = 2 * np.pi * (((R * s1 + s0) * q) % S) / S
    c, s = np.cos(a), np.sin(a)
    fs = np.stack([c, c - s, c + s], 1)
    return np.stack(fw).astype(bf), f0.astype(bf), i0.astype(bf), fs.astype(bf)


_M12, _F0, _I0, _FS = _consts()
_C1, _C2 = float(np.cos(2 * np.pi / 5)), float(np.cos(4 * np.pi / 5))
_S1, _S2 = float(np.sin(2 * np.pi / 5)), float(np.sin(4 * np.pi / 5))
_NT = (((1,), (1,)), ((), ()))


def _dot(a, b):
    return jnp.dot(a, b, preferred_element_type=F32)


def _dot_nt(a, b):
    return jax.lax.dot_general(a, b, _NT, preferred_element_type=F32)


def _dot_tn(a, b):
    return jax.lax.dot_general(a, b, (((0,), (0,)), ((), ())), preferred_element_type=F32)


def _alt(a, b, f_even, f_odd):
    return _cat([(f_odd if i % 2 else f_even)(a[32 * i:32 * i + 32], b[32 * i:32 * i + 32]) for i in range(4)], 0)


def _lhs7(a11, a12, a21, a22):
    return [a11 + a22, a21 + a22, a11, a22, a11 + a12, a21 - a11, a12 - a22]


def _rhs7(b11, b12, b21, b22):
    return [b11 + b22, b11, b12 - b22, b21 - b11, b22, b11 + b12, b21 + b22]


def _chain(*gens):
    for g in gens:
        yield from g


def _pace(gen, n_items, n_slots):
    for sl in range(n_slots):
        for _ in range((n_items * (sl + 1)) // n_slots - (n_items * sl) // n_slots):
            next(gen)
        yield


def _unpack(w):
    return pltpu.bitcast(w << 16, F32), pltpu.bitcast(w & jnp.uint32(0xFFFF0000), F32)


def _cat(xs, axis):
    return jnp.concatenate(xs, axis=axis)


def _cmulc(z, n, N, sign):
    n = (n * sign) % N
    re, im = z
    if n == 0: return re, im
    if 4 * n == N: return -im, re
    if 2 * n == N: return -re, -im
    if 4 * n == 3 * N: return im, -re
    c = float(np.cos(2 * np.pi * n / N)); s = float(np.sin(2 * np.pi * n / N))
    if (8 * n) % N == 0:
        if c * s > 0: return (re - im) * c, (re + im) * c
        return (re + im) * c, (im - re) * c
    return re * c - im * s, re * s + im * c


def _fft(zs, sign):
    n = len(zs)
    if n == 1: return zs
    if n == 2:
        (ar, ai), (br, bi) = zs
        return [(ar + br, ai + bi), (ar - br, ai - bi)]
    if n == 4:
        (ar, ai), (br, bi), (cr, ci), (dr, di) = zs
        t0r, t0i = ar + cr, ai + ci; t1r, t1i = ar - cr, ai - ci
        t2r, t2i = br + dr, bi + di; t3r, t3i = br - dr, bi - di
        p = (t1r + t3i, t1i - t3r); m = (t1r - t3i, t1i + t3r)
        if sign > 0: p, m = m, p
        return [(t0r + t2r, t0i + t2i), p, (t0r - t2r, t0i - t2i), m]
    n1 = 4; n2 = n // 4
    sub = [_fft([zs[n2 * a + b] for a in range(n1)], sign) for b in range(n2)]
    out = [None] * n
    for c in range(n1):
        o = _fft([_cmulc(sub[b][c], b * c, n, sign) for b in range(n2)], sign)
        for e in range(n2): out[c + n1 * e] = o[e]
    return out


def _silu(t):
    u = 0.5 * t
    return u + u * jnp.tanh(u)


def _kernel(x_hbm, wr_hbm, wi_hbm, wg_hbm, wu_hbm, wd_hbm, m12_hbm, f0_hbm, i0_hbm, fs_hbm, o_hbm,
            x_v, xs_v, wr_v, wi_v, nr_v, ni_v, wgu_v, wd_v, m12_v, f0_v, i0_v, fs_v,
            m_v, o_v, acc_v, s_v, sx, sw, so, sf, s0_):
    xi = x_hbm.bitcast(U32)
    oi = o_hbm.bitcast(U32)
    cp = pltpu.make_async_copy
    def xcp(p):
        return cp(xi.at[:, p, :], x_v.at[p], sx.at[p])
    def ocp(p):
        return cp(o_v.at[p], oi.at[:, p, :], so.at[p])
    def fscp(p):
        return cp(fs_hbm.at[pl.ds(2 * p, 2)], fs_v.at[pl.ds(2 * p, 2)], sf.at[p])
    def make_fcps(f):
        return ([cp(w.at[:, pl.ds(n * 128, 128)], wgu_v.at[u, n], sw.at[f] if f else s0_.at[n])
                 for n in range(4 * f, 4 * f + 4) for u, w in enumerate((wg_hbm, wu_hbm))]
                + [cp(wd_hbm.at[pl.ds(512 * f, 512), pl.ds(t * 128, 128)], wd_v.at[f, t], sw.at[f]) for t in range(5)])
    fcps = [make_fcps(f) for f in range(3)]
    ccps = [cp(m12_hbm, m12_v, sw.at[3]), cp(f0_hbm, f0_v, sw.at[3]), cp(i0_hbm, i0_v, sw.at[3])]
    wcps = [cp(a.at[pl.ds(0, 320)].bitcast(U32).at[:, pl.ds(k1 * P, P)], b.at[k1, pl.ds(0, 160)], sw.at[4])
            for a, b in ((wr_hbm, wr_v), (wi_hbm, wi_v)) for k1 in range(R)]
    wcps += [cp(a.at[pl.ds(320, 1), :], b, sw.at[4]) for a, b in ((wr_hbm, nr_v), (wi_hbm, ni_v))]

    xcp(0).start()
    for c in fcps[0][:4]: c.start()

    def blk(base, r, n=8):
        b = base + r // 2
        return pl.ds(b if isinstance(b, int) else pl.multiple_of(b, 8), n)

    def norm(p):
        for r in range(0, P, 16):
            xn = []
            for x in _unpack(x_v[p, r:r + 16, :]):
                xc = x - jnp.mean(x, axis=-1, keepdims=True)
                v = jnp.mean(xc * xc, axis=-1, keepdims=True)
                xn.append(xc * jax.lax.rsqrt(v + 1e-5))
            a12, a21 = xn[0][:, 256:512], xn[1][:, :256]
            ls = _lhs7(xn[0][:, :256], a12, a21, xn[1][:, 256:512]) + [_cat([xn[0][:, 512:], xn[1][:, 512:]], 1), a12, a21]
            for q, t in enumerate(ls):
                t = pltpu.bitcast(t.astype(BF), U32)
                xs_v[blk(640 * p + 64 * q, r), :] = t
                if q < 8: m_v[blk(XS0 + 640 * p + 64 * q, r), :] = t

    def ldxn(p):
        a11, a22, x4, a12, a21 = [pltpu.bitcast(xs_v[blk(640 * p + 64 * q, 0, 64), :], BF) for q in (2, 3, 7, 8, 9)]
        return _cat([_cat([a11, a12, x4[:, :128]], 1), _cat([a21, a22, x4[:, 128:]], 1)], 0)

    def ldrows(ref, bases, side):
        if side is None:
            return _cat([pltpu.bitcast(ref[blk(b, 0, 64), :], BF) for b in bases], 0)
        rows = []
        for b in bases:
            for r in range(0, P, 16):
                next(side)
                rows.append(pltpu.bitcast(ref[blk(b, r), :], BF))
        return _cat(rows, 0)

    def ldxs(f, j, q, side):
        return ldrows(m_v if f == 1 else xs_v, [(XS0 if f == 1 else 0) + 640 * (2 * j + p) + 64 * q for p in range(2)], side)

    def prep(f, i=None, t=None):
        for r in range(0, 256, 16):
            ld = lambda ref, r0: ref[r0 + r:r0 + r + 16, :].astype(F32)
            if t is None:
                n = 4 * f + i - i % 2
                g, u = wgu_v.at[i % 2, n], wgu_v.at[i % 2, n + 1]
                bs, slot = _rhs7(ld(g, 0), ld(u, 0), ld(g, 256), ld(u, 256)), i
            else:
                d0, d1 = wd_v.at[f, 2 * t], wd_v.at[f, 2 * t + 1]
                bs, slot = _rhs7(ld(d0, 0), ld(d1, 0), ld(d0, 256), ld(d1, 256)), 4 + t
            for h2, qq in enumerate((0, 2, 3, 5, 6)):
                ref, at = wm_at(f, slot, h2, r, 16)
                ref[at] = pltpu.bitcast(bs[qq].astype(BF), U32)
            yield

    def wm_at(f, slot, h2, r, n):
        base = (WS0 if f == 2 else 5120 + 1920 * f) + 64 * (5 * slot + h2)
        return (m_v if f == 2 else xs_v), (blk(base, r % 128, n // 2), pl.ds(128 * (r // 128), 128))

    def ldws(f, slot, q):
        if q == 1:
            return wgu_v[slot % 2, 4 * f + slot - slot % 2, :256, :] if slot < 4 else wd_v[f, 2 * slot - 8, :256, :]
        if q == 4:
            return wgu_v[slot % 2, 4 * f + slot - slot % 2 + 1, 256:512, :] if slot < 4 else wd_v[f, 2 * slot - 7, 256:, :]
        h2 = (0, 2, 3, 5, 6).index(q)
        return _cat([pltpu.bitcast(ref[at], BF) for ref, at in (wm_at(f, slot, h2, r, 128) for r in (0, 128))], 0)

    def stage_a(j, HP):
        xn = _cat([ldxn(HP // 2 * j + p) for p in range(HP // 2)], 0).astype(F32)
        x0, x1, x2, x3, x4 = [xn[:, 128 * i:128 * i + 128] for i in range(5)]
        t1, t2, t3, t4 = x1 + x4, x2 + x3, x1 - x4, x2 - x3
        y0 = (x0 + t1 + t2).astype(BF)
        re, im = [], []
        yield
        for cl, (yr, yi) in enumerate(((x0 + _C1 * t1 + _C2 * t2, -_S1 * t3 - _S2 * t4),
                                       (x0 + _C2 * t1 + _C1 * t2, _S1 * t4 - _S2 * t3))):
            k1 = _dot_nt(m12_v[3 * cl], (yr + yi).astype(BF))
            re.append(k1 - _dot_nt(m12_v[3 * cl + 1], yi.astype(BF)))
            im.append(_alt(k1, _dot_nt(m12_v[3 * cl + 2], yr.astype(BF)), lambda p, q: p - q, lambda p, q: q - p))
            yield
        c = _dot_nt(f0_v[...], y0)
        re = _cat(re + [c[:80]], 0)
        im = _cat(im + [c[80:]], 0)
        for h in range(HP):
            yield
            s0 = HP * j + h
            tr, ti = re[:, h * P:h * P + P], im[:, h * P:h * P + P]
            k1 = _dot((tr + ti).astype(BF), fs_v[s0, 0])
            m_v[blk(KR * s0, 0, KR), :P] = pltpu.bitcast(k1 - _dot(ti.astype(BF), fs_v[s0, 1]), U32)
            m_v[blk(KR * s0, 0, KR), P:] = pltpu.bitcast(k1 - _dot(tr.astype(BF), fs_v[s0, 2]), U32)

    def ldp(s0, r0):
        return pltpu.bitcast(m_v[blk(KR * s0 + r0, 0), :P], F32), pltpu.bitcast(m_v[blk(KR * s0 + r0, 0), P:], F32)

    def stp(s0, r0, z):
        m_v[blk(KR * s0 + r0, 0), :P] = pltpu.bitcast(z[0], U32)
        m_v[blk(KR * s0 + r0, 0), P:] = pltpu.bitcast(z[1], U32)

    def stage_m(t, nyq=False):
        r0 = 16 * t
        halves = (0,) if nyq else (0, 8)
        u = t // 2
        res = jnp.where(u < 4, (0x9641 >> (4 * (u & 3))) & 15, jnp.where(u < 8, (0x8732 >> (4 * (u & 3))) & 15, 5 * (u - 8)))
        start = res // 2 + 80 * (t % 2)
        sh = (16 - 16 * (res % 2)).astype(jnp.uint32)
        def ldw(k1, e8):
            if nyq:
                return tuple(w[:, k1 * P:k1 * P + P].astype(F32) for w in (nr_v, ni_v))
            return tuple(pltpu.bitcast((w[k1, pl.ds(start + 5 * e8, 8, stride=5), :] << sh) & U32(0xFFFF0000), F32) for w in (wr_v, wi_v))
        units = [(b, e8) for b in range(4) for e8 in halves]
        for u0 in range(0, len(units), 2):
            us = units[u0:u0 + 2]
            zs = [_fft([ldp(4 * i + b, r0 + e8) for i in range(4)], -1) for b, e8 in us]
            for (b, e8), z in zip(us, zs):
                for c in range(4): stp(4 * c + b, r0 + e8, _cmulc(z[c], b * c, R, -1))
            yield
        for u0 in range(0, len(units), 1):
            us = units[u0:u0 + 1]
            zs = [_fft([ldp(4 * c + b, r0 + e8) for b in range(4)], -1) for c, e8 in us]
            for (c, e8), z in zip(us, zs):
                w = [ldw(c + 4 * e, e8) for e in range(4)]
                z = _fft([(zr * wr - zi * wi, zr * wi + zi * wr) for (zr, zi), (wr, wi) in zip(z, w)], 1)
                for b in range(4): stp(4 * c + b, r0 + e8, _cmulc(z[b], b * c, R, 1))
            yield
        for b in range(4):
            z = [_fft([ldp(4 * c + b, r0 + e8) for c in range(4)], 1) for e8 in halves]
            if nyq: z.append([(jnp.zeros((8, P), F32),) * 2] * 4)
            for i in range(4):
                zr, zi = _cat([z[0][i][0], z[1][i][0]], 0), _cat([z[0][i][1], z[1][i][1]], 0)
                q0 = 8 * t
                m_v[blk(KR * (R + 4 * i + b) + q0, 0), :] = pltpu.bitcast(_cat([zr, zi], 1).astype(BF), U32)
                m_v[blk(KR * (R + 4 * i + b) + KR // 2 + q0, 0), :P] = pltpu.bitcast((zr + zi).astype(BF), U32)
            yield

    def ffn_plain(p, first=False, mid=None):
        xn = lambda: ldxn(p)
        if first:
            waits = (fcps[0][:2], fcps[0][2:4], fcps[0][4:8] + ccps + [fscp(0)], [])
            starts = (fcps[0][6:8] + ccps + [fscp(0)], fcps[0][8:] + [xcp(1)], [], [])
        hs = []
        for n in range(4):
            if first:
                for c in waits[n]: c.wait()
                for c in starts[n]: c.start()
                if n % 2:
                    for _ in _chain(prep(0, i=n - 1), prep(0, i=n)): pass
            if mid is not None: next(mid, None)
            g = _silu(_dot(xn(), wgu_v[0, n]))
            if mid is not None: next(mid, None)
            hs.append((g * _dot(xn(), wgu_v[1, n])).astype(BF))
        if mid is not None:
            for _ in mid: pass
        if first:
            for c in (xcp(2), fscp(1), xcp(3), xcp(4), xcp(5), fscp(2)): c.start()
            for c in fcps[0][8:] + [xcp(1)]: c.wait()
            norm(1)
            for _ in _chain(prep(0, t=0), prep(0, t=1)): pass
        return _dot(_cat(hs, 1), _cat([wd_v[0, t] for t in range(5)], 1)).reshape(2, P, D)

    def ffn(f, j, side=None, mid=None):
        order = (0, 3, 4, 6, 2, 1, 5)
        hs = []
        for i in range(4):
            if mid is not None: next(mid, None)
            x4 = ldxs(f, j, 7, side)
            x4 = _cat([x4[:, :128], x4[:, 128:]], 0)
            g4, u4 = [_dot(x4, wgu_v[i % 2, 4 * f + i - i % 2 + e, 512:, :]) for e in range(2)]
            m1, m4 = [_dot(ldxs(f, j, q, side), ldws(f, i, q)) for q in order[:2]]
            if mid is not None: next(mid, None)
            m5, m7, m3, m2, m6 = [_dot(ldxs(f, j, q, side), ldws(f, i, q)) for q in order[2:]]
            c = _cat([_cat([g4[:256] + m1 + m4 - m5 + m7, u4[:256] + m3 + m5], 1),
                      _cat([g4[256:] + m2 + m4, u4[256:] + m1 - m2 + m3 + m6], 1)], 0)
            hs.append(hs.pop().astype(F32) * c if i % 2 else _silu(c).astype(BF))
        if mid is not None:
            for _ in mid: pass
        h = _cat(hs, 1)
        a12, a21 = h[:256, 256:], h[256:, :256]
        ls = [t.astype(BF) for t in _lhs7(h[:256, :256], a12, a21, h[256:, 256:])]
        cols = []
        for t in range(2):
            m1, m4, m5, m7, m3, m2, m6 = [_dot(ls[q], ldws(f, 4 + t, q)) for q in order]
            cols += [_cat([m1 + m4 - m5 + m7, m2 + m4], 0), _cat([m3 + m5, m1 - m2 + m3 + m6], 0)]
        cols.append(_dot(_cat([_cat([ls[2], a12.astype(BF)], 1), _cat([a21.astype(BF), ls[3]], 1)], 0), wd_v[f, 4]))
        y = _cat(cols, 1)
        return _cat([y[0:128], y[256:384], y[128:256], y[384:512]], 0).reshape(4, P, D)

    def stage_c(j, HP):
        zr, zi = [], []
        for h in range(HP):
            s0 = HP * j + h
            k1 = _dot_nt(pltpu.bitcast(m_v[blk(KR * (R + s0) + KR // 2, 0, KR // 2), :P], BF), fs_v[s0, 0])
            zr.append(k1 - _dot_nt(pltpu.bitcast(m_v[blk(KR * (R + s0), 0, KR // 2), P:], BF), fs_v[s0, 2]))
            zi.append(k1 - _dot_nt(pltpu.bitcast(m_v[blk(KR * (R + s0), 0, KR // 2), :P], BF), fs_v[s0, 1]))
            yield
        yield
        zr, zi = _cat(zr, 1), _cat(zi, 1)
        us = []
        for cl in range(2):
            ar, ai = zr[128 * cl:128 * cl + 128], zi[128 * cl:128 * cl + 128]
            k1 = _dot_tn(_alt(ar, ai, lambda p, q: p + q, lambda p, q: p - q).astype(BF), m12_v[3 * cl])
            ai = _alt(ar, ai, lambda p, q: q, lambda p, q: -q)
            us += [k1 - _dot_tn(ai.astype(BF), m12_v[3 * cl + 2]), k1 - _dot_tn(ar.astype(BF), m12_v[3 * cl + 1])]
            yield
        u1r, u1i, u2r, u2i = us
        row = jax.lax.broadcasted_iota(jnp.int32, (16, HP * P), 0)
        u0 = _dot_tn(_cat([zr[256:320], jnp.where(row == 0, zr[320:336], zi[256:272]), zi[272:320]], 0).astype(BF), i0_v[...])
        e1 = u0 + _C1 * u1r + _C2 * u2r; o1 = _S1 * u1i + _S2 * u2i
        e2 = u0 + _C2 * u1r + _C1 * u2r; o2 = _S2 * u1i - _S1 * u2i
        s = _cat([u0 + u1r + u2r, e1 - o1, e2 - o2, e2 + o2, e1 + o1], 1)
        s_v[...] = s * (2.0 / (D * S))

    xcp(0).wait()
    for c in fcps[0][4:6]: c.start()
    norm(0)
    acc_v[0:2] = ffn_plain(0, first=True, mid=_chain([None] * 4, stage_a(0, 2)))
    for c in [xcp(6), xcp(7)] + [fscp(p) for p in range(3, 8)]: c.start()

    def l1a(p, _):
        xcp(2 * p).wait()
        xcp(2 * p + 1).wait()
        fscp(p).wait()
        @pl.when(p == 2)
        def _():
            for c in fcps[1]: c.start()
        def after():
            norm(2 * p)
            norm(2 * p + 1)
            yield
        acc_v[pl.ds(2 * p, 2)] = ffn_plain(p, mid=_chain(stage_a(p, 2), [None] * 3, after()))
        return 0
    with jax.named_scope("S_1a"):
        jax.lax.fori_loop(1, 4, l1a, 0)
        for c in wcps + fcps[2]: c.start()
        for c in fcps[1]: c.wait()

    def l1b(j, _):
        fscp(2 * j).wait()
        fscp(2 * j + 1).wait()
        side = _pace(_chain(prep(1, i=2 * j - 4), prep(1, i=2 * j - 3), prep(1, t=j - 2)), 48, 1)
        acc_v[pl.ds(4 * j, 4)] = ffn(0, j, mid=_chain(stage_a(j, 4), [None], side))
        return 0
    with jax.named_scope("S_1b"):
        jax.lax.fori_loop(2, 4, l1b, 0)
        for c in wcps + fcps[2]: c.wait()
    for _ in stage_m(20, nyq=True): pass

    def l2(j, _):
        side = _pace(_chain(prep(2, i=j), prep(2, t=j // 2), *[stage_m(5 * j + i) for i in range(5)]), 5 * 16 + 2 * 16, 4 * 8 * 16)
        acc_v[pl.ds(4 * j, 4)] += ffn(1, j, side=side)
        return 0
    with jax.named_scope("S_l2"):
        jax.lax.fori_loop(0, 4, l2, 0)

    def l3(j, _):
        g = _silu(acc_v[pl.ds(4 * j, 4)] + ffn(2, j, mid=stage_c(j, 4))).reshape(4 * P, D)
        for p in range(2):
            x = _cat(_unpack(x_v[2 * j + p]), 0)
            rows = slice(2 * P * p, 2 * P * p + 2 * P)
            o = pltpu.bitcast((x + s_v[rows] * g[rows]).astype(BF).astype(F32), U32)
            o_v[2 * j + p] = (o[:P] >> 16) | o[P:]
        for p in range(2): ocp(2 * j + p).start()
        return 0
    with jax.named_scope("S_l3"):
        jax.lax.fori_loop(0, 4, l3, 0)
    for p in range(8): ocp(p).wait()


@jax.jit
def pallas_recurrent_scan__spectral_gfnet__swiglu_ffn__prompt_kernel(A_x, A_w_r, A_w_i, B_x, B_w_gate, B_w_up, B_w_down):
    del B_x
    hbm = pl.BlockSpec(memory_space=pltpu.HBM)
    V, SEM = pltpu.VMEM, pltpu.SemaphoreType.DMA
    out = pl.pallas_call(
        _kernel,
        in_specs=[hbm] * 10,
        out_specs=hbm,
        out_shape=jax.ShapeDtypeStruct((P, R, D), BF),
        scratch_shapes=[
            V((8, P, D), U32), V((5120 + 2 * 1920, 256), U32),
            V((R, 168, P), U32), V((R, 168, P), U32), V((1, S), BF), V((1, S), BF),
            V((2, 12, D, 128), BF), V((3, 5, 512, 128), BF),
            V((6, 128, 128), BF), V((160, 128), BF), V((128, 128), BF), V((R, 3, P, P), BF),
            V((M_ROWS, 2 * P), U32), V((8, P, D), U32), V((R, P, D), F32), V((4 * P, D), F32),
            SEM((8,)), SEM((6,)), SEM((8,)), SEM((8,)), SEM((4,)),
        ],
        compiler_params=pltpu.CompilerParams(vmem_limit_bytes=100 * 1024 * 1024,
                                             flags={"XLA_TPU_EVENLY_DISTRIBUTE_CRITICAL_NODES": True}),
    )(A_x.reshape(P, R, D), A_w_r.T, A_w_i.T, B_w_gate, B_w_up, B_w_down, _M12, _F0, _I0, _FS)
    return out.reshape(1, S, D)
```
